```python
import jax
import jax.numpy as jnp

def _softmax(x, axis=-1):
    return jax.nn.softmax(x, axis=axis)
def _gelu(x):
    return jax.nn.gelu(x, approximate=True)
def _silu(x):
    return jax.nn.silu(x)
def _sigmoid(x):
    return jax.nn.sigmoid(x)
def _layernorm(x, axis=-1, eps=1e-5):
    m = jnp.mean(x, axis=axis, keepdims=True)
    v = jnp.var(x, axis=axis, keepdims=True)
    return (x - m) / jnp.sqrt(v + eps)
def _scatter_add(tgt, idx, src, axis=0):
    return tgt.at[idx].add(src)
def _segment_sum(src, seg, n):
    return jax.ops.segment_sum(src, seg, n)
class _Rng:
    def __init__(self, key):
        self._k = key
    def _next(self):
        self._k, sub = jax.random.split(self._k)
        return sub
    def normal(self, shape):
        return jax.random.normal(self._next(), shape, dtype=jnp.bfloat16)
    def randint(self, lo, hi, shape):
        return jax.random.randint(self._next(), shape, lo, hi, dtype=jnp.int32)
    def uniform(self, shape, lo=0.0, hi=1.0):
        return jax.random.uniform(self._next(), shape, jnp.bfloat16, lo, hi)
    def permutation(self, n):
        return jax.random.permutation(self._next(), n)


kernel_name = 'standalone__fused_io_aware_attn__prompt'

def setup_inputs():
    _rng = _Rng(jax.random.key(int.from_bytes(__import__("os").urandom(4), "little")))
    _w = (lambda a: (lambda t: t.astype(jnp.bfloat16) if jnp.issubdtype(t.dtype, jnp.floating) else t)(jnp.asarray(a)))
    B, H, S = 2, 32, 2048
    Dh = max(1, 1024 // 32)
    return {
        "q": _w((lambda *s: _rng.normal(s) * 0.05)(B, H, S, Dh)),
        "k": _w((lambda *s: _rng.normal(s) * 0.05)(B, H, S, Dh)),
        "v": _w((lambda *s: _rng.normal(s) * 0.05)(B, H, S, Dh)),
    }

def reference(q, k, v):
    scale = q.shape[-1] ** -0.5
    s = jnp.einsum('bhqd,bhkd->bhqk', q, k) * scale
    p = _softmax(s, axis=-1)
    return jnp.einsum('bhqk,bhkd->bhqd', p, v)
```

```python
import math

import jax
import jax.numpy as jnp
import jax.experimental.pallas as pl
import jax.experimental.pallas.tpu as pltpu

BQ = 512
BS = 128
LA = 2
HB = 8
U = 2


@jax.jit
def pallas_standalone__fused_io_aware_attn__prompt_kernel(
    q: jax.Array,
    k: jax.Array,
    v: jax.Array,
):
    B, H, S, D = q.shape
    qt = jnp.swapaxes(q, 2, 3).reshape(B * H, D, S)
    kt = jnp.swapaxes(k, 2, 3).reshape(B * H, D, S)
    vt = jnp.swapaxes(v, 2, 3).reshape(B * H, D, S)
    c = (D ** -0.5) * math.log2(math.e)
    nq, nk = S // BQ, S // BS
    f32, bf = jnp.float32, jnp.bfloat16

    def safe(q_ref, k_ref, v_ref, h):
        qs = q_ref[h].astype(f32) * c
        kf = k_ref[h].astype(f32)
        q2 = jnp.max(jnp.sum(qs * qs, axis=0, keepdims=True))
        k2 = jnp.max(jnp.sum(kf * kf, axis=0, keepdims=True))
        vm = jnp.max(jnp.abs(v_ref[h].astype(f32)))
        return (q2 * k2 <= 1600.0) & (vm <= 2.0 ** 60) & (vm >= 2.0 ** -40)

    def fast(q_ref, k_ref, v_ref, o_ref, h0):
        kk = [[k_ref[h0 + u, :, j * BS:(j + 1) * BS].astype(f32).T.astype(bf)
               for j in range(nk)] for u in range(U)]
        qs = [[q_ref[h0 + u, :, i * BQ:(i + 1) * BQ] for i in range(nq)]
              for u in range(U)]
        chunks = [(u, i, j) for u in range(U) for i in range(nq) for j in range(nk)]
        N = len(chunks)
        sv = {}
        l = acc = None
        for n in range(N + LA):
            if n < N:
                u, i, j = chunks[n]
                sv[n] = jnp.dot(kk[u][j], qs[u][i], preferred_element_type=f32)
            if n >= LA:
                u, i, j = chunks[n - LA]
                p = jnp.exp2(sv.pop(n - LA) * c)
                l8 = p.reshape(BS // 8, 8, BQ).sum(0)
                o = jnp.dot(v_ref[h0 + u, :, j * BS:(j + 1) * BS], p.astype(bf),
                            preferred_element_type=f32)
                l = l8 if j == 0 else l + l8
                acc = o if j == 0 else acc + o
                if j == nk - 1:
                    r = 1.0 / jnp.sum(l, axis=0, keepdims=True)
                    o_ref[h0 + u, :, i * BQ:(i + 1) * BQ] = (acc * r).astype(o_ref.dtype)

    def slow(q_ref, k_ref, v_ref, o_ref, h):
        def qtile(i, carry):
            sl = pl.ds(pl.multiple_of(i * BQ, BQ), BQ)
            s = jax.lax.dot_general(k_ref[h], q_ref[h, :, sl], (((0,), (0,)), ((), ())),
                                    preferred_element_type=f32)
            m = jnp.max(s, axis=0, keepdims=True)
            p = jnp.exp2((s - m) * c)
            l = jnp.sum(p, axis=0, keepdims=True)
            o = jnp.dot(v_ref[h], p.astype(bf), preferred_element_type=f32)
            o_ref[h, :, sl] = (o / l).astype(o_ref.dtype)
            return carry
        jax.lax.fori_loop(0, nq, qtile, 0)

    def kern(q_ref, k_ref, v_ref, o_ref, ok_ref):
        def chk(h0):
            ok = safe(q_ref, k_ref, v_ref, h0)
            for u in range(1, U):
                ok = ok & safe(q_ref, k_ref, v_ref, h0 + u)
            return ok.astype(jnp.int32)

        ok_ref[0] = chk(0)

        def body(g, carry):
            h0 = g * U
            nxt = jnp.minimum(h0 + U, HB - U)
            ok = ok_ref[0]

            @pl.when(ok == 1)
            def _():
                fast(q_ref, k_ref, v_ref, o_ref, h0)
                ok_ref[0] = chk(nxt)

            @pl.when(ok != 1)
            def _():
                def hb(u, cc):
                    slow(q_ref, k_ref, v_ref, o_ref, h0 + u)
                    return cc
                jax.lax.fori_loop(0, U, hb, 0)
                ok_ref[0] = chk(nxt)

            return carry
        jax.lax.fori_loop(0, HB // U, body, 0)

    spec = pl.BlockSpec((HB, D, S), lambda h: (h, 0, 0))
    o = pl.pallas_call(
        kern,
        grid=(B * H // HB,),
        in_specs=[spec, spec, spec],
        out_specs=spec,
        out_shape=jax.ShapeDtypeStruct((B * H, D, S), q.dtype),
        scratch_shapes=[pltpu.SMEM((1,), jnp.int32)],
        compiler_params=pltpu.CompilerParams(
            dimension_semantics=("parallel",), vmem_limit_bytes=100 * 1024 * 1024),
    )(qt, kt, vt)
    return jnp.swapaxes(o.reshape(B, H, D, S), 2, 3)
```
